```python
import jax
import jax.numpy as jnp

def _softmax(x, axis=-1):
    return jax.nn.softmax(x, axis=axis)
def _gelu(x):
    return jax.nn.gelu(x, approximate=True)
def _silu(x):
    return jax.nn.silu(x)
def _sigmoid(x):
    return jax.nn.sigmoid(x)
def _layernorm(x, axis=-1, eps=1e-5):
    m = jnp.mean(x, axis=axis, keepdims=True)
    v = jnp.var(x, axis=axis, keepdims=True)
    return (x - m) / jnp.sqrt(v + eps)
def _scatter_add(tgt, idx, src, axis=0):
    return tgt.at[idx].add(src)
def _segment_sum(src, seg, n):
    return jax.ops.segment_sum(src, seg, n)
class _Rng:
    def __init__(self, key):
        self._k = key
    def _next(self):
        self._k, sub = jax.random.split(self._k)
        return sub
    def normal(self, shape):
        return jax.random.normal(self._next(), shape, dtype=jnp.bfloat16)
    def randint(self, lo, hi, shape):
        return jax.random.randint(self._next(), shape, lo, hi, dtype=jnp.int32)
    def uniform(self, shape, lo=0.0, hi=1.0):
        return jax.random.uniform(self._next(), shape, jnp.bfloat16, lo, hi)
    def permutation(self, n):
        return jax.random.permutation(self._next(), n)


kernel_name = 'parallel_sum__sliding_block_cached__mixer_s_mlp__decode'

def setup_inputs():
    _rng = _Rng(jax.random.key(int.from_bytes(__import__("os").urandom(4), "little")))
    _w = (lambda a: (lambda t: t.astype(jnp.bfloat16) if jnp.issubdtype(t.dtype, jnp.floating) else t)(jnp.asarray(a)))
    def _A_setup():
        B, Sq, D = 4, 1, 512
        Hq, Hkv, Sk, Dh = 32, 32, 8192, 128
        assert Hq % Hkv == 0, (Hq, Hkv)
        return {
            "x": _w((lambda *s: _rng.normal(s) * 0.05)(B, Sq, D)),
            "k_cache": _w((lambda *s: _rng.normal(s) * 0.05)(B, Hkv, Sk, Dh)),
            "v_cache": _w((lambda *s: _rng.normal(s) * 0.05)(B, Hkv, Sk, Dh)),
            "wq": _w((lambda *s: _rng.normal(s) * 0.05)(D, Hq * Dh) * (D ** -0.5)),
            "wo": _w((lambda *s: _rng.normal(s) * 0.05)(Hq * Dh, D) * ((Hq * Dh) ** -0.5)),
        }
    _A_in = _A_setup()

    def _B_setup():
        B, S, D, F = 4, 1, 512, 1376
        return {
            "x":  _w((lambda *s: _rng.normal(s) * 0.05)(B, S, D)),
            "w1": _w((lambda *s: _rng.normal(s) * 0.05)(D, D) * (D ** -0.5)),
            "w2": _w((lambda *s: _rng.normal(s) * 0.05)(D, D) * (D ** -0.5)),
            "w3": _w((lambda *s: _rng.normal(s) * 0.05)(D, F) * (D ** -0.5)),
            "w4": _w((lambda *s: _rng.normal(s) * 0.05)(F, D) * (F ** -0.5)),
        }
    _B_in = _B_setup()

    return {
        "A_x": _A_in["x"],
        "A_k_cache": _A_in["k_cache"],
        "A_v_cache": _A_in["v_cache"],
        "A_wq": _A_in["wq"],
        "A_wo": _A_in["wo"],
        "B_x": _B_in["x"],
        "B_w1": _B_in["w1"],
        "B_w2": _B_in["w2"],
        "B_w3": _B_in["w3"],
        "B_w4": _B_in["w4"],
    }

def reference(A_x, A_k_cache, A_v_cache, A_wq, A_wo, B_x, B_w1, B_w2, B_w3, B_w4):
    def _A_ref(x, k_cache, v_cache, wq, wo):
        B, Sq, D = x.shape
        Hq, Dh = 32, 128
        Hkv, Sk = k_cache.shape[1], k_cache.shape[2]
        W = min(4096, max(256, Sk // 4))
        rep = Hq // Hkv
        q = (lambda x, *d: x.transpose(*d))((x @ wq).reshape(B, Sq, Hq, Dh), 0, 2, 1, 3)
        k = jnp.repeat(k_cache[:, :, Sk - W:, :], rep, axis=1)
        v = jnp.repeat(v_cache[:, :, Sk - W:, :], rep, axis=1)
        scores = jnp.einsum("bhqd,bhkd->bhqk", q, k) * (Dh ** -0.5)
        p = _softmax(scores, axis=-1)
        o = jnp.einsum("bhqk,bhkd->bhqd", p, v)
        return (lambda x, *d: x.transpose(*d))(o, 0, 2, 1, 3).reshape(B, Sq, Hq * Dh) @ wo

    def _B_ref(x, w1, w2, w3, w4):
        B, S, D = x.shape
        h = _gelu(_layernorm(x, axis=-1) @ w1)
        c = D // 4
        g0 = jnp.pad(h[:, :, 0*c:1*c], ((0, 0), (1, 0), (0, 0)))[:, :S, :]
        g1 = jnp.pad(h[:, :, 1*c:2*c], ((0, 0), (0, 1), (0, 0)))[:, 1:, :]
        g2 = jnp.pad(h[:, :, 2*c:3*c], ((0, 0), (2, 0), (0, 0)))[:, :S, :]
        g3 = jnp.pad(h[:, :, 3*c:   ], ((0, 0), (0, 2), (0, 0)))[:, 2:, :]
        hs = jnp.concatenate([g0, g1, g2, g3], axis=-1) @ w2
        x1 = x + hs
        h2 = _gelu(_layernorm(x1, axis=-1) @ w3) @ w4
        return x1 + h2

    x = A_x
    xn = _layernorm(x, axis=-1)
    return x + _A_ref(xn, A_k_cache, A_v_cache, A_wq, A_wo) + _B_ref(xn, B_w1, B_w2, B_w3, B_w4)
```

```python
import functools

import jax
import jax.numpy as jnp
from jax import lax
import jax.experimental.pallas as pl
import jax.experimental.pallas.tpu as pltpu

F32 = jnp.float32
BF16 = jnp.bfloat16
NT = (((1,), (1,)), ((), ()))


def _layernorm(x):
    m = jnp.mean(x, axis=-1, keepdims=True)
    d = x - m
    v = jnp.mean(d * d, axis=-1, keepdims=True)
    return d / jnp.sqrt(v + 1e-5)


def make(LOOK=4, NSLOT=8, nocompute=False):
    B, D, H, DH, SK, F = 4, 512, 32, 128, 8192, 1376
    W = 2048
    W0 = SK - W
    CH = 512
    NC = W // CH
    PR = 128
    NP = CH // PR
    T = H * NC

    def kern(x_hbm, k_hbm, v_hbm, wq_hbm, wo_hbm, w3_hbm, w4_hbm, o_hbm,
             x_v, wq_v, wo_v, w3_v, w4_v, kbuf, vbuf, xn_s, q_s, s_s, p_s, l_s, o_s, acc_s, h_s, out_v,
             sem, wsem, ksem, vsem):
        def piece(src, buf, sems, t, j, b):
            h = t // NC
            r = pl.multiple_of(W0 + lax.rem(t, NC) * CH + j * PR, PR)
            slot = lax.rem(t, NSLOT)
            return pltpu.make_async_copy(
                src.at[b, h, pl.ds(r, PR), :], buf.at[slot, b, pl.ds(j * PR, PR), :], sems.at[slot])

        kp = functools.partial(piece, k_hbm, kbuf, ksem)
        vp = functools.partial(piece, v_hbm, vbuf, vsem)

        xc = pltpu.make_async_copy(x_hbm, x_v, sem.at[0])
        xc.start()

        def w_issue(i, _):
            for s in range(4):
                g = i + s * 32
                r = pl.multiple_of((g // 4) * 16, 16)
                c = pl.multiple_of(lax.rem(g, 4) * 1024, 1024)
                pltpu.make_async_copy(wq_hbm.at[pl.ds(r, 16), pl.ds(c, 1024)],
                                      wq_v.at[pl.ds(r, 16), pl.ds(c, 1024)], wsem.at[0]).start(priority=0)
                r = pl.multiple_of(g * 32, 32)
                pltpu.make_async_copy(wo_hbm.at[pl.ds(r, 32), :], wo_v.at[pl.ds(r, 32), :],
                                      wsem.at[1]).start(priority=1)
        lax.fori_loop(0, 32, w_issue, None)

        def m_issue(i, _):
            r = pl.multiple_of(i * 32, 32)
            pltpu.make_async_copy(w3_hbm.at[pl.ds(r, 32), :], w3_v.at[pl.ds(r, 32), :],
                                  wsem.at[2]).start(priority=0)
            pltpu.make_async_copy(w4_hbm.at[pl.ds(r, 32), :], w4_v.at[pl.ds(r, 32), :],
                                  wsem.at[3]).start(priority=1)
        lax.fori_loop(0, F // 32, m_issue, None)

        def k0_issue(i, _):
            for j in range(NP):
                for b in range(B):
                    kp(i + NC // 2, j, b).start(priority=0)
                    kp(i, j, b).start(priority=1)
        lax.fori_loop(0, NC // 2, k0_issue, None)

        xc.wait()
        x = x_v[...].astype(F32)
        xn = _layernorm(x).astype(BF16)
        xn_s[...] = xn
        acc_s[...] = x + xn.astype(F32)
        pltpu.make_async_copy(wq_hbm, wq_v, wsem.at[0]).wait()

        def q_head(h):
            c = pl.multiple_of(h * DH, DH)
            q = jnp.dot(xn_s[...], wq_v[:, pl.ds(c, DH)], preferred_element_type=F32)
            q_s[...] = q.astype(BF16)

        q_head(0)
        row = lax.broadcasted_iota(jnp.int32, (B, DH), 0)
        rowc = lax.broadcasted_iota(jnp.int32, (B, CH), 0)

        def step(tt, _):
            t = tt - NC
            tk = tt
            c = lax.rem(tt, NC)
            ti = t + LOOK

            @pl.when(ti < T - NC)
            def _():
                for j in range(NP):
                    for b in range(B):
                        kp(ti + NC, j, b).start(priority=0)
                        vp(ti, j, b).start(priority=1)

            @pl.when((ti >= T - NC // 2) & (ti < T))
            def _():
                for j in range(NP):
                    for b in range(B):
                        vp(ti - NC // 2, j, b).start(priority=0)
                        vp(ti, j, b).start(priority=1)

            @pl.when(tt == 0)
            def _():
                pltpu.make_async_copy(w3_hbm, w3_v, wsem.at[2]).wait()
                x2 = _layernorm(xn_s[...].astype(F32)).astype(BF16)
                hh = lax.dot_general(x2, w3_v[...], NT, preferred_element_type=F32)
                h_s[...] = jax.nn.gelu(hh, approximate=True).astype(BF16)

            @pl.when(tt == 1)
            def _():
                pltpu.make_async_copy(w4_hbm, w4_v, wsem.at[3]).wait()
                pltpu.make_async_copy(wo_hbm, wo_v, wsem.at[1]).wait()
                acc_s[...] += jnp.dot(h_s[...], w4_v[...], preferred_element_type=F32)

            @pl.when(tk < T)
            def _():
                slot = lax.rem(tk, NSLOT)
                pltpu.make_async_copy(kbuf.at[slot], kbuf.at[slot], ksem.at[slot]).wait()
                if not nocompute:
                    q = q_s[...]
                    s = None
                    for b in range(B):
                        sb = lax.dot_general(q, kbuf[slot, b], NT, preferred_element_type=F32)
                        s = sb if s is None else jnp.where(rowc == b, sb, s)
                    s_s[c] = s * (DH ** -0.5)

            @pl.when(t >= 0)
            def _():
                slot = lax.rem(t, NSLOT)
                pltpu.make_async_copy(vbuf.at[slot], vbuf.at[slot], vsem.at[slot]).wait()
                if not nocompute:
                    p = p_s[c]
                    o = None
                    for b in range(B):
                        ob = jnp.dot(p, vbuf[slot, b], preferred_element_type=F32)
                        o = ob if o is None else jnp.where(row == b, ob, o)
                    o_s[...] += o

            @pl.when(c == NC - 1)
            def _():
                @pl.when(t >= 0)
                def _():
                    o = (o_s[...] / l_s[...]).astype(BF16)
                    r = pl.multiple_of((t // NC) * DH, DH)
                    acc_s[...] += jnp.dot(o, wo_v[pl.ds(r, DH), :], preferred_element_type=F32)

                @pl.when(tk < T)
                def _():
                    ss = [s_s[i] for i in range(NC)]
                    m = functools.reduce(jnp.maximum, ss)
                    m = jnp.max(m, axis=-1, keepdims=True)
                    ps = [jnp.exp(s - m) for s in ss]
                    for i in range(NC):
                        p_s[i] = ps[i].astype(BF16)
                    l = jnp.sum(functools.reduce(jnp.add, ps), axis=-1, keepdims=True)
                    l_s[...] = jnp.broadcast_to(l, (B, DH))
                    o_s[...] = jnp.zeros((B, DH), F32)
                    q_head(jnp.minimum(tk // NC + 1, H - 1))

        lax.fori_loop(0, T + NC, step, None)
        out_v[...] = acc_s[...].astype(BF16)
        oc = pltpu.make_async_copy(out_v, o_hbm, sem.at[1])
        oc.start()
        oc.wait()

    def f(A_x, A_k_cache, A_v_cache, A_wq, A_wo, B_x, B_w1, B_w2, B_w3, B_w4):
        anys = pl.BlockSpec(memory_space=pl.ANY)
        out = pl.pallas_call(
            kern,
            out_shape=jax.ShapeDtypeStruct((B, D), BF16),
            in_specs=[anys] * 7,
            out_specs=anys,
            scratch_shapes=[
                pltpu.VMEM((B, D), BF16),
                pltpu.VMEM((D, H * DH), BF16),
                pltpu.VMEM((H * DH, D), BF16),
                pltpu.VMEM((F, D), BF16),
                pltpu.VMEM((F, D), BF16),
                pltpu.VMEM((NSLOT, B, CH, DH), BF16),
                pltpu.VMEM((NSLOT, B, CH, DH), BF16),
                pltpu.VMEM((B, D), BF16),
                pltpu.VMEM((B, DH), BF16),
                pltpu.VMEM((NC, B, CH), F32),
                pltpu.VMEM((NC, B, CH), BF16),
                pltpu.VMEM((B, DH), F32),
                pltpu.VMEM((B, DH), F32),
                pltpu.VMEM((B, D), F32),
                pltpu.VMEM((B, F), BF16),
                pltpu.VMEM((B, D), BF16),
                pltpu.SemaphoreType.DMA((2,)),
                pltpu.SemaphoreType.DMA((4,)),
                pltpu.SemaphoreType.DMA((NSLOT,)),
                pltpu.SemaphoreType.DMA((NSLOT,)),
            ],
            compiler_params=pltpu.CompilerParams(
                vmem_limit_bytes=64 * 1024 * 1024, disable_bounds_checks=True),
            name="attn_mlp_kernel",
        )(A_x.reshape(B, D), A_k_cache, A_v_cache, A_wq, A_wo, B_w3.T, B_w4)
        return out.reshape(B, 1, D)
    return f


_impl = make()


@jax.jit
def pallas_parallel_sum__sliding_block_cached__mixer_s_mlp__decode_kernel(
    A_x, A_k_cache, A_v_cache, A_wq, A_wo, B_x, B_w1, B_w2, B_w3, B_w4,
):
    return _impl(A_x, A_k_cache, A_v_cache, A_wq, A_wo, B_x, B_w1, B_w2, B_w3, B_w4)
```

```python
import functools

import jax
import jax.numpy as jnp
from jax import lax
import jax.experimental.pallas as pl
import jax.experimental.pallas.tpu as pltpu

F32 = jnp.float32
BF16 = jnp.bfloat16
NT = (((1,), (1,)), ((), ()))


def _layernorm(x):
    m = jnp.mean(x, axis=-1, keepdims=True)
    d = x - m
    v = jnp.mean(d * d, axis=-1, keepdims=True)
    return d / jnp.sqrt(v + 1e-5)


def make(NSLOT=8, nocompute=False, offk=0, offv=1, offq=0, offo=0, off3=0, off4=0, wqmode="8x2048",
         mlpmix=True, now=False, nomlp=False, scopes=False, semchk=False):
    B, D, H, DH, SK, F = 4, 512, 32, 128, 8192, 1376
    W = 2048
    W0 = SK - W
    CH = 512
    NC = W // CH
    PR = 128
    HP = PR // 2
    NP = CH // PR
    T = H * NC
    RING = NSLOT * CH

    def kern(x_hbm, k_hbm, v_hbm, wq_hbm, wo_hbm, w3_hbm, w4_hbm, o_hbm,
             x_v, wq_v, wo_v, w3_v, w4_v, kbuf, vbuf, xn_s, q_s, s_s, p_s, l_s, o_s, acc_s, h_s, out_v,
             sem, wsem, ksem, vsem):
        def piece(src, buf, sems, off, t, j, b, prio):
            h = t >> 2
            c = t & (NC - 1)
            slot = t & (NSLOT - 1)

            def full():
                r = pl.multiple_of(W0 + c * CH + j * PR + off * HP, HP)
                d = pl.multiple_of(slot * CH + j * PR + off * HP, HP)
                pltpu.make_async_copy(src.at[b, h, pl.ds(r, PR), :], buf.at[b, pl.ds(d, PR), :],
                                      sems.at[slot]).start(priority=prio)
            if not off or j < NP - 1:
                full()
                return
            pl.when(c != NC - 1)(full)

            @pl.when(c == NC - 1)
            def _():
                b2 = (b % 2) * 2
                if b < 2:
                    d = pl.multiple_of(slot * CH + CH - HP, HP)
                    pltpu.make_async_copy(src.at[pl.ds(b2, 2), h, pl.ds(SK - HP, HP), :],
                                          buf.at[pl.ds(b2, 2), pl.ds(d, HP), :], sems.at[slot]).start(priority=prio)
                else:
                    @pl.when(h < H - 1)
                    def _():
                        head_piece(src, buf, sems.at[slot], h + 1, b2, prio)

        def head_piece(src, buf, s, h, b2, prio):
            d = pl.multiple_of(((h * NC) & (NSLOT - 1)) * CH, CH)
            pltpu.make_async_copy(src.at[pl.ds(b2, 2), h, pl.ds(W0, HP), :],
                                  buf.at[pl.ds(b2, 2), pl.ds(d, HP), :], s).start(priority=prio)

        def wait_group(buf, sems, off, t):
            slot = t & (NSLOT - 1)

            def w(n):
                pltpu.make_async_copy(buf.at[:, pl.ds(0, n), :], buf.at[:, pl.ds(0, n), :], sems.at[slot]).wait()
            if not off:
                w(CH)
            else:
                w(CH - HP)
                pl.when(t != T - 1)(lambda: w(HP))
                pl.when(t == 0)(lambda: w(HP))

        kp = functools.partial(piece, k_hbm, kbuf, ksem, offk)
        vp = functools.partial(piece, v_hbm, vbuf, vsem, offv)

        xc = pltpu.make_async_copy(x_hbm, x_v, sem.at[0])
        xc.start()

        def rows_piece(src, dst, s, off, g, n, prio):
            def full():
                r = pl.multiple_of(g * 32 + off * 16, 16)
                pltpu.make_async_copy(src.at[pl.ds(r, 32), :], dst.at[pl.ds(r, 32), :], s).start(priority=prio)
            if not off:
                full()
                return
            pl.when(g != n - 1)(full)

            @pl.when(g == n - 1)
            def _():
                for r in (0, n * 32 - 16):
                    pltpu.make_async_copy(src.at[pl.ds(r, 16), :], dst.at[pl.ds(r, 16), :], s).start(priority=prio)

        def wq_piece(i, s):
            g = i + s * 32
            if wqmode == "16x1024":
                r = pl.multiple_of((g >> 2) * 16, 16)
                c = pl.multiple_of((g & 3) * 1024, 1024)
                pltpu.make_async_copy(wq_hbm.at[pl.ds(r, 16), pl.ds(c, 1024)],
                                      wq_v.at[pl.ds(r, 16), pl.ds(c, 1024)], wsem.at[0]).start(priority=0)
            elif not offq:
                r = pl.multiple_of((g >> 1) * 8, 8)
                c = pl.multiple_of((g & 1) * 2048, 2048)
                pltpu.make_async_copy(wq_hbm.at[pl.ds(r, 8), pl.ds(c, 2048)],
                                      wq_v.at[pl.ds(r, 8), pl.ds(c, 2048)], wsem.at[0]).start(priority=0)
            else:
                r = pl.multiple_of((g >> 1) * 8, 8)

                @pl.when((g & 1) == 0)
                def _():
                    pltpu.make_async_copy(wq_hbm.at[pl.ds(r, 8), pl.ds(1024, 2048)],
                                          wq_v.at[pl.ds(r, 8), pl.ds(1024, 2048)], wsem.at[0]).start(priority=0)

                @pl.when((g & 1) == 1)
                def _():
                    r2 = pl.multiple_of((r + 8) & (D - 1), 8)
                    pltpu.make_async_copy(wq_hbm.at[pl.ds(r, 8), pl.ds(3072, 1024)],
                                          wq_v.at[pl.ds(r, 8), pl.ds(3072, 1024)], wsem.at[0]).start(priority=0)
                    pltpu.make_async_copy(wq_hbm.at[pl.ds(r2, 8), pl.ds(0, 1024)],
                                          wq_v.at[pl.ds(r2, 8), pl.ds(0, 1024)], wsem.at[0]).start(priority=0)

        def m_pair(i):
            rows_piece(w3_hbm, w3_v, wsem.at[2], off3, i, F // 32, 0)
            rows_piece(w4_hbm, w4_v, wsem.at[3], off4, i, F // 32, 1)

        def w_issue(i, _):
            for s in range(4):
                wq_piece(i, s)
                rows_piece(wo_hbm, wo_v, wsem.at[1], offo, i + s * 32, 128, 1)
                if mlpmix and s == 1:
                    pl.when(i < F // 32 - 32)(lambda: m_pair(i + 32))
            if mlpmix:
                m_pair(i)
        if not now: lax.fori_loop(0, 32, w_issue, None)
        if not mlpmix:
            lax.fori_loop(0, F // 32, lambda i, _: m_pair(i), None)

        for b2 in (0, 2):
            if offk:
                head_piece(k_hbm, kbuf, ksem.at[0], 0, b2, b2 // 2)
            if offv:
                head_piece(v_hbm, vbuf, vsem.at[0], 0, b2, b2 // 2)

        def k0_issue(i, _):
            for j in range(NP):
                for b in range(B):
                    kp(i + NC // 2, j, b, 0)
                    kp(i, j, b, 1)
        lax.fori_loop(0, NC // 2, k0_issue, None)

        xc.wait()
        x = x_v[...].astype(F32)
        xn = _layernorm(x).astype(BF16)
        xn_s[...] = xn
        acc_s[...] = x + xn.astype(F32)
        if not now: pltpu.make_async_copy(wq_hbm, wq_v, wsem.at[0]).wait()

        def q_head(h):
            c = pl.multiple_of(h * DH, DH)
            q = jnp.dot(xn_s[...], wq_v[:, pl.ds(c, DH)], preferred_element_type=F32)
            q_s[...] = q.astype(BF16)

        q_head(0)
        row = lax.broadcasted_iota(jnp.int32, (B, DH), 0)
        rowc = lax.broadcasted_iota(jnp.int32, (B, CH), 0)

        def step(tt, _):
            t = tt - NC
            tk = tt
            c = tt & (NC - 1)
            ti = tt

            @pl.when(ti < T - NC)
            def _():
                for j in range(NP):
                    for b in range(B):
                        kp(ti + NC, j, b, 0)
                        vp(ti, j, b, 1)

            @pl.when((ti >= T - NC // 2) & (ti < T))
            def _():
                for j in range(NP):
                    for b in range(B):
                        vp(ti - NC // 2, j, b, 0)
                        vp(ti, j, b, 1)

            @pl.when(tt == 0)
            def _():
                if not now: pltpu.make_async_copy(w3_hbm, w3_v, wsem.at[2]).wait()
                if nomlp: return
                x2 = _layernorm(xn_s[...].astype(F32)).astype(BF16)
                hh = lax.dot_general(x2, w3_v[...], NT, preferred_element_type=F32)
                h_s[...] = jax.nn.gelu(hh, approximate=True).astype(BF16)

            @pl.when(tt == 1)
            def _():
                if not now: pltpu.make_async_copy(w4_hbm, w4_v, wsem.at[3]).wait()
                if not now: pltpu.make_async_copy(wo_hbm, wo_v, wsem.at[1]).wait()
                if nomlp: return
                acc_s[...] += jnp.dot(h_s[...], w4_v[...], preferred_element_type=F32)

            @pl.when(tk < T)
            def _():
                wait_group(kbuf, ksem, offk, tk)
                if not nocompute:
                    r = pl.multiple_of((tk & (NSLOT - 1)) * CH, CH)
                    q = q_s[...]
                    s = None
                    for b in range(B):
                        sb = lax.dot_general(q, kbuf[b, pl.ds(r, CH), :], NT, preferred_element_type=F32)
                        s = sb if s is None else jnp.where(rowc == b, sb, s)
                    s_s[c] = s * (DH ** -0.5)

            @pl.when(t >= 0)
            def _():
                wait_group(vbuf, vsem, offv, t)
                if not nocompute:
                    r = pl.multiple_of((t & (NSLOT - 1)) * CH, CH)
                    p = p_s[c]
                    o = None
                    for b in range(B):
                        ob = jnp.dot(p, vbuf[b, pl.ds(r, CH), :], preferred_element_type=F32)
                        o = ob if o is None else jnp.where(row == b, ob, o)
                    o_s[...] += o

            @pl.when(c == NC - 1)
            def _():
                @pl.when(t >= 0)
                def _():
                    o = (o_s[...] / l_s[...]).astype(BF16)
                    r = pl.multiple_of((t >> 2) * DH, DH)
                    acc_s[...] += jnp.dot(o, wo_v[pl.ds(r, DH), :], preferred_element_type=F32)

                @pl.when(tk < T)
                def _():
                    ss = [s_s[i] for i in range(NC)]
                    m = functools.reduce(jnp.maximum, ss)
                    m = jnp.max(m, axis=-1, keepdims=True)
                    ps = [jnp.exp(s - m) for s in ss]
                    for i in range(NC):
                        p_s[i] = ps[i].astype(BF16)
                    l = jnp.sum(functools.reduce(jnp.add, ps), axis=-1, keepdims=True)
                    l_s[...] = jnp.broadcast_to(l, (B, DH))
                    o_s[...] = jnp.zeros((B, DH), F32)
                    q_head(jnp.minimum((tk >> 2) + 1, H - 1))

        lax.fori_loop(0, T + NC, step, None)
        out_v[...] = acc_s[...].astype(BF16)
        oc = pltpu.make_async_copy(out_v, o_hbm, sem.at[1])
        oc.start()
        oc.wait()

    def f(A_x, A_k_cache, A_v_cache, A_wq, A_wo, B_x, B_w1, B_w2, B_w3, B_w4):
        anys = pl.BlockSpec(memory_space=pl.ANY)
        out = pl.pallas_call(
            kern,
            out_shape=jax.ShapeDtypeStruct((B, D), BF16),
            in_specs=[anys] * 7,
            out_specs=anys,
            scratch_shapes=[
                pltpu.VMEM((B, D), BF16),
                pltpu.VMEM((D, H * DH), BF16),
                pltpu.VMEM((H * DH, D), BF16),
                pltpu.VMEM((F, D), BF16),
                pltpu.VMEM((F, D), BF16),
                pltpu.VMEM((B, RING, DH), BF16),
                pltpu.VMEM((B, RING, DH), BF16),
                pltpu.VMEM((B, D), BF16),
                pltpu.VMEM((B, DH), BF16),
                pltpu.VMEM((NC, B, CH), F32),
                pltpu.VMEM((NC, B, CH), BF16),
                pltpu.VMEM((B, DH), F32),
                pltpu.VMEM((B, DH), F32),
                pltpu.VMEM((B, D), F32),
                pltpu.VMEM((B, F), BF16),
                pltpu.VMEM((B, D), BF16),
                pltpu.SemaphoreType.DMA((2,)),
                pltpu.SemaphoreType.DMA((4,)),
                pltpu.SemaphoreType.DMA((NSLOT,)),
                pltpu.SemaphoreType.DMA((NSLOT,)),
            ],
            compiler_params=pltpu.CompilerParams(
                vmem_limit_bytes=64 * 1024 * 1024, disable_bounds_checks=True, disable_semaphore_checks=not semchk),
            name="attn_mlp_kernel",
        )(A_x.reshape(B, D), A_k_cache, A_v_cache, A_wq, A_wo, B_w3.T, B_w4)
        return out.reshape(B, 1, D)
    return f


_impl = make()


@jax.jit
def pallas_parallel_sum__sliding_block_cached__mixer_s_mlp__decode_kernel(
    A_x, A_k_cache, A_v_cache, A_wq, A_wo, B_x, B_w1, B_w2, B_w3, B_w4,
):
    return _impl(A_x, A_k_cache, A_v_cache, A_wq, A_wo, B_x, B_w1, B_w2, B_w3, B_w4)
```

```python
import functools

import jax
import jax.numpy as jnp
from jax import lax
import jax.experimental.pallas as pl
import jax.experimental.pallas.tpu as pltpu

F32 = jnp.float32
BF16 = jnp.bfloat16
NT = (((1,), (1,)), ((), ()))


def _layernorm(x):
    m = jnp.mean(x, axis=-1, keepdims=True)
    d = x - m
    v = jnp.mean(d * d, axis=-1, keepdims=True)
    return d / jnp.sqrt(v + 1e-5)


def make(NSLOT=8, LOOK=5, offv=1, nocompute=False, head=3, scopes=False, stages=(5, 2, 1)):
    import contextlib
    sc = (lambda n: jax.named_scope(n)) if scopes else (lambda n: contextlib.nullcontext())
    B, D, H, DH, SK, F = 4, 512, 32, 128, 8192, 1376
    W = 2048
    W0 = SK - W
    NS = 16
    NG = B * H // NS
    HG = NS // B
    CH = 256
    NC = W // CH
    PR = 128
    HP = PR // 2
    T = NG * 2 * NC
    FT = 2 * NS * 32
    ends = [sum(stages[:i + 1]) for i in range(len(stages))]

    def srow(s):
        return (s % HG) * B + s // HG

    def kern(x_hbm, k_hbm, v_hbm, wq_hbm, wo_hbm, w3_hbm, w4_hbm, o_hbm,
             x_v, wq_v, wo_v, w3_v, w4_v, buf, xn_s, q_s, s_s, p_s, r_s, o_s, acc_s, res_s, h_s, out_v,
             sem, wsem, osem, bsem):
        def rows_copy(src, dst, s, r, n):
            return pltpu.make_async_copy(src.at[pl.ds(r, n), :], dst.at[pl.ds(r, n), :], s)

        def full_piece(src, g, r, slot, j, s):
            return pltpu.make_async_copy(src.at[s, g, pl.ds(r + j * PR, PR), :],
                                         buf.at[slot, s, pl.ds(j * PR, PR), :], bsem.at[slot])

        def half_piece(src, g, slot, s):
            s2 = (s // 2) * 2
            r, d = ((SK - HP, CH - PR), (W0, CH - HP))[s % 2]
            return pltpu.make_async_copy(src.at[pl.ds(s2, 2), g, pl.ds(r, HP), :],
                                         buf.at[slot, pl.ds(s2, 2), pl.ds(d, HP), :], bsem.at[slot])

        def slab(mk):
            for s in range(NS // 2):
                mk(s).start(priority=0)
                mk(s + NS // 2).start(priority=1)

        def issue(t):
            g = t >> 4
            c = t & (NC - 1)
            slot = t & (NSLOT - 1)

            @pl.when((t & NC) == 0)
            def _():
                r = pl.multiple_of(W0 + c * CH, CH)
                for j in range(CH // PR):
                    slab(functools.partial(full_piece, k_hbm, g, r, slot, j))

            @pl.when((t & NC) != 0)
            def _():
                r = pl.multiple_of(W0 + c * CH + offv * HP, HP)
                full = functools.partial(full_piece, v_hbm, g, r, slot, CH // PR - 1)
                last = functools.partial(half_piece, v_hbm, g, slot) if offv else full
                first = functools.partial(full_piece, v_hbm, g, r, slot, 0)

                @pl.when(t != T - 1)
                def _():
                    slab(first)
                    pl.when(c != NC - 1)(lambda: slab(full))
                    pl.when(c == NC - 1)(lambda: slab(last))

                @pl.when(t == T - 1)
                def _():
                    for n in range(2 * NS):
                        (first, last)[n // NS](n % NS).start(priority=0)
                        st = sum(n >= 4 * e for e in ends)
                        rows_copy(w4_hbm, w4_v, osem.at[st], n * 32, 32).start(priority=1)

        xc = pltpu.make_async_copy(x_hbm, x_v, sem.at[0])
        with sc("s_x"):
            xc.start()

        def wq_piece(g):
            r = pl.multiple_of((g >> 1) * 8, 8)
            c = pl.multiple_of((g & 1) * 2048, 2048)
            return pltpu.make_async_copy(wq_hbm.at[pl.ds(r, 8), pl.ds(c, 2048)],
                                         wq_v.at[pl.ds(r, 8), pl.ds(c, 2048)], wsem.at[0])

        def m_piece(src, dst, s, i, p):
            rows_copy(src, dst, s, pl.multiple_of(i * 32, 32), 32).start(priority=p)

        def w_issue(p0, i, _):
            for s in (0, 2, 1, 3):
                rows_copy(wo_hbm, wo_v, wsem.at[1], pl.multiple_of((i + s * 32) * 32, 32), 32).start(priority=1)
                wq_piece(i + s * 32).start(priority=p0)
                if s == 2:
                    @pl.when(i < 11)
                    def _():
                        m_piece(w4_hbm, w4_v, wsem.at[3], i + 32, 1)
                        m_piece(w3_hbm, w3_v, wsem.at[2], i + 16, p0)

            @pl.when(i >= 16)
            def _():
                m_piece(w3_hbm, w3_v, wsem.at[2], i - 16, 1)
                m_piece(w3_hbm, w3_v, wsem.at[2], i + 11, p0)

        if head:
            lax.fori_loop(0, head, functools.partial(w_issue, 1), None)
        lax.fori_loop(head, 32, functools.partial(w_issue, 0), None)

        lax.fori_loop(0, LOOK, lambda t, _: issue(t), None)

        xc.wait()
        x = x_v[...].astype(F32)
        xn = _layernorm(x).astype(BF16).astype(F32)
        xn_s[...] = jnp.concatenate([xn] * HG, axis=0).astype(BF16)
        res_s[...] = x + xn
        acc_s[...] = jnp.zeros(acc_s.shape, F32)
        pltpu.make_async_copy(wq_hbm, wq_v, wsem.at[0]).wait()

        def rows(n):
            return lax.broadcasted_iota(jnp.int32, (NS, n), 0)

        def pick(vals, n):
            r8 = lax.broadcasted_iota(jnp.int32, (8, n), 0)
            out = [None, None]
            for s, v in enumerate(vals):
                hi, lo = divmod(srow(s), 8)
                v = v[hi * 8:(hi + 1) * 8]
                out[hi] = v if out[hi] is None else jnp.where(r8 == lo, v, out[hi])
            return jnp.concatenate(out, axis=0)

        def wait(t):
            slot = t & (NSLOT - 1)
            pltpu.make_async_copy(buf.at[slot], buf.at[slot], bsem.at[slot]).wait()
            return slot

        def step(t, _):
            g = t >> 4
            c = t & (NC - 1)
            pl.when(t + LOOK < T)(lambda: issue(t + LOOK))

            @pl.when(t == 1)
            def _():
                pltpu.make_async_copy(w3_hbm, w3_v, wsem.at[2]).wait()
                x2 = _layernorm(xn_s[...].astype(F32)).astype(BF16)
                hh = lax.dot_general(x2, w3_v[...], NT, preferred_element_type=F32)
                h_s[...] = jax.nn.gelu(hh, approximate=True).astype(BF16)

            @pl.when(t == 2)
            def _():
                rows_copy(w4_hbm, w4_v, wsem.at[3], FT, F - FT).wait()
                pltpu.make_async_copy(wo_hbm, wo_v, wsem.at[1]).wait()
                res_s[...] += jnp.dot(h_s[:, FT:], w4_v[FT:, :], preferred_element_type=F32)[:B]

            @pl.when((t & (2 * NC - 1)) == 0)
            def _():
                q = None
                for hh in range(HG):
                    col = pl.multiple_of((g + NG * hh) * DH, DH)
                    qh = jnp.dot(xn_s[...], wq_v[:, pl.ds(col, DH)], preferred_element_type=F32)
                    q = qh if q is None else jnp.where(rows(DH) >= hh * B, qh, q)
                q_s[...] = q.astype(BF16)

            @pl.when((t & (2 * NC - 1)) == NC)
            def _():
                s = jnp.concatenate([s_s[i] for i in range(NC)], axis=1)
                p = jnp.exp(s - jnp.max(s, axis=-1, keepdims=True))
                r_s[...] = jnp.broadcast_to(1.0 / jnp.sum(p, axis=-1, keepdims=True), (NS, DH))
                if offv:
                    p = pltpu.roll(p, W - HP, 1)
                p = p.astype(BF16)
                for i in range(NC):
                    p_s[i] = p[:, i * CH:(i + 1) * CH]
                o_s[...] = jnp.zeros(o_s.shape, F32)

            with sc("s_wait"):
                slot = wait(t)
            if nocompute:
                return

            @pl.when((t & NC) == 0)
            def _():
                q = q_s[...]
                s = [lax.dot_general(q, buf[slot, i], NT, preferred_element_type=F32) for i in range(NS)]
                s_s[c] = pick(s, CH) * (DH ** -0.5)

            @pl.when((t & NC) != 0)
            def _():
                p = p_s[c]
                o = [jnp.dot(p, buf[slot, i], preferred_element_type=F32) for i in range(NS)]
                o_s[...] += pick(o, DH)

            @pl.when((t & (2 * NC - 1)) == 2 * NC - 1)
            def _():
                o = (o_s[...] * r_s[...]).astype(BF16)
                a = None
                for hh in range(HG):
                    r = pl.multiple_of((g + NG * hh) * DH, DH)
                    ah = jnp.dot(o, wo_v[pl.ds(r, DH), :], preferred_element_type=F32)
                    a = ah if a is None else jnp.where(rows(D) >= hh * B, ah, a)
                acc_s[...] += a

        lax.fori_loop(0, T, step, None)

        a = acc_s[...]
        res = res_s[...]
        for hh in range(HG):
            res += a[hh * B:(hh + 1) * B]
        for st, e in enumerate(ends):
            r, n = (e - stages[st]) * 128, stages[st] * 128
            with sc(f"s_wo{st}"):
                rows_copy(w4_hbm, w4_v, osem.at[st], r, n).wait()
            res += jnp.dot(h_s[:, r:r + n], w4_v[r:r + n, :], preferred_element_type=F32)[:B]
        out_v[...] = res.astype(BF16)
        oc = pltpu.make_async_copy(out_v, o_hbm, sem.at[1])
        with sc("s_out"):
            oc.start()
            oc.wait()

    def f(A_x, A_k_cache, A_v_cache, A_wq, A_wo, B_x, B_w1, B_w2, B_w3, B_w4):
        anys = pl.BlockSpec(memory_space=pl.ANY)
        out = pl.pallas_call(
            kern,
            out_shape=jax.ShapeDtypeStruct((B, D), BF16),
            in_specs=[anys] * 7,
            out_specs=anys,
            scratch_shapes=[
                pltpu.VMEM((B, D), BF16),
                pltpu.VMEM((D, H * DH), BF16),
                pltpu.VMEM((H * DH, D), BF16),
                pltpu.VMEM((F, D), BF16),
                pltpu.VMEM((F, D), BF16),
                pltpu.VMEM((NSLOT, NS, CH, DH), BF16),
                pltpu.VMEM((NS, D), BF16),
                pltpu.VMEM((NS, DH), BF16),
                pltpu.VMEM((NC, NS, CH), F32),
                pltpu.VMEM((NC, NS, CH), BF16),
                pltpu.VMEM((NS, DH), F32),
                pltpu.VMEM((NS, DH), F32),
                pltpu.VMEM((NS, D), F32),
                pltpu.VMEM((B, D), F32),
                pltpu.VMEM((NS, F), BF16),
                pltpu.VMEM((B, D), BF16),
                pltpu.SemaphoreType.DMA((2,)),
                pltpu.SemaphoreType.DMA((4,)),
                pltpu.SemaphoreType.DMA((len(stages),)),
                pltpu.SemaphoreType.DMA((NSLOT,)),
            ],
            compiler_params=pltpu.CompilerParams(
                vmem_limit_bytes=64 * 1024 * 1024, disable_bounds_checks=True, disable_semaphore_checks=True),
            name="attn_mlp_kernel",
        )(A_x.reshape(B, D), A_k_cache.reshape(NS, NG, SK, DH), A_v_cache.reshape(NS, NG, SK, DH),
          A_wq, A_wo, B_w3.T, B_w4)
        return out.reshape(B, 1, D)
    return f


_impl = make()


@jax.jit
def pallas_parallel_sum__sliding_block_cached__mixer_s_mlp__decode_kernel(
    A_x, A_k_cache, A_v_cache, A_wq, A_wo, B_x, B_w1, B_w2, B_w3, B_w4,
):
    return _impl(A_x, A_k_cache, A_v_cache, A_wq, A_wo, B_x, B_w1, B_w2, B_w3, B_w4)
```

```python
import functools

import jax
import jax.numpy as jnp
from jax import lax
import jax.experimental.pallas as pl
import jax.experimental.pallas.tpu as pltpu

F32 = jnp.float32
BF16 = jnp.bfloat16
NT_DIMS = (((1,), (1,)), ((), ()))

B, D, H, DH, SK, F = 4, 512, 32, 128, 8192, 1376
W = min(4096, max(256, SK // 4))
W0 = SK - W

NS = 16
NG = B * H // NS
HG = NS // B
PR = 128
HP = PR // 2
CH = 2 * PR
NC = W // CH
STEPS = NG * 2 * NC
NSLOT = 8
LOOKAHEAD = 5
WR = 32
W4_TAIL = 2 * NS * WR
TAIL_ENDS = (640, 896, W4_TAIL)
RAMP = 3


def _layernorm(x):
    d = x - jnp.mean(x, axis=-1, keepdims=True)
    var = jnp.mean(d * d, axis=-1, keepdims=True)
    return d / jnp.sqrt(var + 1e-5)


def _row_ids(shape):
    return lax.broadcasted_iota(jnp.int32, shape, 0)


def _pick_window_rows(vals):
    ids = _row_ids((8, vals[0].shape[1]))
    out = [None, None]
    for s, v in enumerate(vals):
        hi, lo = divmod((s % HG) * B + s // HG, 8)
        v = v[hi * 8:(hi + 1) * 8]
        out[hi] = v if out[hi] is None else jnp.where(ids == lo, v, out[hi])
    return jnp.concatenate(out, axis=0)


def _pick_head_rows(vals):
    out = vals[0]
    for hh in range(1, HG):
        out = jnp.where(_row_ids(out.shape) >= hh * B, vals[hh], out)
    return out


def _kernel(x_hbm, k_hbm, v_hbm, wq_hbm, wo_hbm, w3t_hbm, w4_hbm, out_hbm,
            x_v, wq_v, wo_v, w3t_v, w4_v, ring, xn_s, q_s, s_s, p_s, inv_s, o_s, att_s, res_s, h_s, out_v,
            io_sem, w_sem, tail_sem, ring_sem):

    def rows_copy(src, dst, sem, start, size):
        return pltpu.make_async_copy(src.at[pl.ds(start, size), :], dst.at[pl.ds(start, size), :], sem)

    def weight_piece(src, dst, sem, i):
        return rows_copy(src, dst, sem, pl.multiple_of(i * WR, WR), WR)

    def wq_piece(i):
        r = pl.ds(pl.multiple_of((i >> 1) * 8, 8), 8)
        c = pl.ds(pl.multiple_of((i & 1) * 2048, 2048), 2048)
        return pltpu.make_async_copy(wq_hbm.at[r, c], wq_v.at[r, c], w_sem.at[0])

    def kv_piece(src, g, row, slot, j, s):
        return pltpu.make_async_copy(src.at[s, g, pl.ds(row + j * PR, PR), :],
                                     ring.at[slot, s, pl.ds(j * PR, PR), :], ring_sem.at[slot])

    def v_wrap_piece(g, slot, s):
        pair = pl.ds((s // 2) * 2, 2)
        row, dst = ((SK - HP, PR), (W0, PR + HP))[s % 2]
        return pltpu.make_async_copy(v_hbm.at[pair, g, pl.ds(row, HP), :],
                                     ring.at[slot, pair, pl.ds(dst, HP), :], ring_sem.at[slot])

    def start_slab(piece):
        for s in range(NS // 2):
            piece(s).start(priority=0)
            piece(s + NS // 2).start(priority=1)

    def issue(t):
        g = t // (2 * NC)
        c = t & (NC - 1)
        slot = t & (NSLOT - 1)

        @pl.when((t & NC) == 0)
        def _():
            row = pl.multiple_of(W0 + c * CH, CH)
            start_slab(functools.partial(kv_piece, k_hbm, g, row, slot, 0))
            start_slab(functools.partial(kv_piece, k_hbm, g, row, slot, 1))

        @pl.when((t & NC) != 0)
        def _():
            row = pl.multiple_of(W0 + c * CH + HP, HP)
            first = functools.partial(kv_piece, v_hbm, g, row, slot, 0)
            second = functools.partial(kv_piece, v_hbm, g, row, slot, 1)
            wrap = functools.partial(v_wrap_piece, g, slot)

            @pl.when(t != STEPS - 1)
            def _():
                start_slab(first)
                pl.when(c != NC - 1)(lambda: start_slab(second))
                pl.when(c == NC - 1)(lambda: start_slab(wrap))

            @pl.when(t == STEPS - 1)
            def _():
                for n in range(2 * NS):
                    (first, wrap)[(n // 8) % 2](n % 8 + (n // NS) * 8).start(priority=0)
                    stage = sum(n * WR >= end for end in TAIL_ENDS)
                    rows_copy(w4_hbm, w4_v, tail_sem.at[stage], n * WR, WR).start(priority=1)

    def issue_weights(prio, i, _):
        for quarter in (0, 2, 1, 3):
            weight_piece(wo_hbm, wo_v, w_sem.at[1], i + quarter * 32).start(priority=1)
            wq_piece(i + quarter * 32).start(priority=prio)
            if quarter == 2:
                @pl.when(i < 11)
                def _():
                    weight_piece(w4_hbm, w4_v, w_sem.at[3], i + W4_TAIL // WR).start(priority=1)
                    weight_piece(w3t_hbm, w3t_v, w_sem.at[2], i + 16).start(priority=prio)

        @pl.when(i >= 16)
        def _():
            weight_piece(w3t_hbm, w3t_v, w_sem.at[2], i - 16).start(priority=1)
            weight_piece(w3t_hbm, w3t_v, w_sem.at[2], i + 11).start(priority=prio)

    lax.fori_loop(0, RAMP, functools.partial(issue_weights, 1), None)
    x_copy = pltpu.make_async_copy(x_hbm, x_v, io_sem.at[0])
    x_copy.start()
    lax.fori_loop(RAMP, 32, functools.partial(issue_weights, 0), None)
    lax.fori_loop(0, LOOKAHEAD, lambda t, _: issue(t), None)

    x_copy.wait()
    x = x_v[...].astype(F32)
    xn = _layernorm(x).astype(BF16).astype(F32)
    xn_s[...] = jnp.concatenate([xn] * HG, axis=0).astype(BF16)
    res_s[...] = x + xn
    att_s[...] = jnp.zeros(att_s.shape, F32)
    pltpu.make_async_copy(wq_hbm, wq_v, w_sem.at[0]).wait()

    def step(t, _):
        g = t // (2 * NC)
        c = t & (NC - 1)
        phase = t & (2 * NC - 1)
        slot = t & (NSLOT - 1)

        def head_slice(hh):
            return pl.ds(pl.multiple_of((g + NG * hh) * DH, DH), DH)

        pl.when(t + LOOKAHEAD < STEPS)(lambda: issue(t + LOOKAHEAD))

        @pl.when(t == 1)
        def _():
            pltpu.make_async_copy(w3t_hbm, w3t_v, w_sem.at[2]).wait()
            x2 = _layernorm(xn_s[...].astype(F32)).astype(BF16)
            h = lax.dot_general(x2, w3t_v[...], NT_DIMS, preferred_element_type=F32)
            h_s[...] = jax.nn.gelu(h, approximate=True).astype(BF16)

        @pl.when(t == 2)
        def _():
            rows_copy(w4_hbm, w4_v, w_sem.at[3], W4_TAIL, F - W4_TAIL).wait()
            pltpu.make_async_copy(wo_hbm, wo_v, w_sem.at[1]).wait()
            res_s[...] += jnp.dot(h_s[:, W4_TAIL:], w4_v[W4_TAIL:, :], preferred_element_type=F32)[:B]

        @pl.when(phase == 0)
        def _():
            q = [jnp.dot(xn_s[...], wq_v[:, head_slice(hh)], preferred_element_type=F32) for hh in range(HG)]
            q_s[...] = _pick_head_rows(q).astype(BF16)

        @pl.when(phase == NC)
        def _():
            s = jnp.concatenate([s_s[i] for i in range(NC)], axis=1)
            p = jnp.exp(s - jnp.max(s, axis=-1, keepdims=True))
            inv_s[...] = jnp.broadcast_to(1.0 / jnp.sum(p, axis=-1, keepdims=True), inv_s.shape)
            p = pltpu.roll(p, W - HP, 1).astype(BF16)
            for i in range(NC):
                p_s[i] = p[:, i * CH:(i + 1) * CH]
            o_s[...] = jnp.zeros(o_s.shape, F32)

        pltpu.make_async_copy(ring.at[slot], ring.at[slot], ring_sem.at[slot]).wait()

        @pl.when(phase < NC)
        def _():
            q = q_s[...]
            s = [lax.dot_general(q, ring[slot, i], NT_DIMS, preferred_element_type=F32) for i in range(NS)]
            s_s[c] = _pick_window_rows(s) * (DH ** -0.5)

        @pl.when(phase >= NC)
        def _():
            p = p_s[c]
            o = [jnp.dot(p, ring[slot, i], preferred_element_type=F32) for i in range(NS)]
            o_s[...] += _pick_window_rows(o)

        @pl.when(phase == 2 * NC - 1)
        def _():
            o = (o_s[...] * inv_s[...]).astype(BF16)
            a = [jnp.dot(o, wo_v[head_slice(hh), :], preferred_element_type=F32) for hh in range(HG)]
            att_s[...] += _pick_head_rows(a)

    lax.fori_loop(0, STEPS, step, None)

    att = att_s[...]
    res = res_s[...]
    for hh in range(HG):
        res += att[hh * B:(hh + 1) * B]
    res = jnp.concatenate([res, res], axis=0)
    for stage, (lo, hi) in enumerate(zip((0,) + TAIL_ENDS, TAIL_ENDS)):
        rows_copy(w4_hbm, w4_v, tail_sem.at[stage], lo, hi - lo).wait()
        res += jnp.dot(h_s[:, lo:hi], w4_v[lo:hi, :], preferred_element_type=F32)[:2 * B]
    out_v[...] = res.astype(out_v.dtype)[:B]
    out_copy = pltpu.make_async_copy(out_v, out_hbm, io_sem.at[1])
    out_copy.start()
    out_copy.wait()


@jax.jit
def pallas_parallel_sum__sliding_block_cached__mixer_s_mlp__decode_kernel(
    A_x: jax.Array,
    A_k_cache: jax.Array,
    A_v_cache: jax.Array,
    A_wq: jax.Array,
    A_wo: jax.Array,
    B_x: jax.Array,
    B_w1: jax.Array,
    B_w2: jax.Array,
    B_w3: jax.Array,
    B_w4: jax.Array,
):
    assert A_x.shape == (B, 1, D), A_x.shape
    assert A_k_cache.shape == A_v_cache.shape == (B, H, SK, DH)
    assert B_w3.shape == (D, F) and B_w4.shape == (F, D)
    del B_x, B_w1, B_w2

    in_hbm = pl.BlockSpec(memory_space=pl.ANY)
    out = pl.pallas_call(
        _kernel,
        out_shape=jax.ShapeDtypeStruct((B, D), A_x.dtype),
        in_specs=[in_hbm] * 7,
        out_specs=in_hbm,
        scratch_shapes=[
            pltpu.VMEM((B, D), BF16),
            pltpu.VMEM((D, H * DH), BF16),
            pltpu.VMEM((H * DH, D), BF16),
            pltpu.VMEM((F, D), BF16),
            pltpu.VMEM((F, D), BF16),
            pltpu.VMEM((NSLOT, NS, CH, DH), BF16),
            pltpu.VMEM((NS, D), BF16),
            pltpu.VMEM((NS, DH), BF16),
            pltpu.VMEM((NC, NS, CH), F32),
            pltpu.VMEM((NC, NS, CH), BF16),
            pltpu.VMEM((NS, DH), F32),
            pltpu.VMEM((NS, DH), F32),
            pltpu.VMEM((NS, D), F32),
            pltpu.VMEM((B, D), F32),
            pltpu.VMEM((NS, F), BF16),
            pltpu.VMEM((B, D), BF16),
            pltpu.SemaphoreType.DMA((2,)),
            pltpu.SemaphoreType.DMA((4,)),
            pltpu.SemaphoreType.DMA((len(TAIL_ENDS),)),
            pltpu.SemaphoreType.DMA((NSLOT,)),
        ],
        compiler_params=pltpu.CompilerParams(
            vmem_limit_bytes=64 * 1024 * 1024,
            disable_semaphore_checks=True,
        ),
        name="pallas_parallel_sum__sliding_block_cached__mixer_s_mlp__decode_kernel",
    )(
        A_x.reshape(B, D),
        A_k_cache.reshape(NS, NG, SK, DH),
        A_v_cache.reshape(NS, NG, SK, DH),
        A_wq,
        A_wo,
        B_w3.T,
        B_w4,
    )
    return out.reshape(B, 1, D)
```
